```python
import jax
import jax.numpy as jnp

def _softmax(x, axis=-1):
    return jax.nn.softmax(x, axis=axis)

def _gelu(x):
    return jax.nn.gelu(x, approximate=True)

def _silu(x):
    return jax.nn.silu(x)

def _sigmoid(x):
    return jax.nn.sigmoid(x)

def _layernorm(x, axis=-1, eps=1e-05):
    m = jnp.mean(x, axis=axis, keepdims=True)
    v = jnp.var(x, axis=axis, keepdims=True)
    return (x - m) / jnp.sqrt(v + eps)

def _scatter_add(tgt, idx, src, axis=0):
    return tgt.at[idx].add(src)

def _segment_sum(src, seg, n):
    return jax.ops.segment_sum(src, seg, n)

class _Rng:

    def __init__(self, key):
        self._k = key

    def _next(self):
        self._k, sub = jax.random.split(self._k)
        return sub

    def normal(self, shape):
        return jax.random.normal(self._next(), shape, dtype=jnp.bfloat16)

    def randint(self, lo, hi, shape):
        return jax.random.randint(self._next(), shape, lo, hi, dtype=jnp.int32)

    def uniform(self, shape, lo=0.0, hi=1.0):
        return jax.random.uniform(self._next(), shape, jnp.bfloat16, lo, hi)

    def permutation(self, n):
        return jax.random.permutation(self._next(), n)
kernel_name = 'standalone__window_attn_davit__vision'

def setup_inputs():
    _rng = _Rng(jax.random.key(int.from_bytes(__import__("os").urandom(4), "little")))
    _w = lambda a: (lambda t: t.astype(jnp.bfloat16) if jnp.issubdtype(t.dtype, jnp.floating) else t)(jnp.asarray(a))
    HW = 512
    C0 = 192
    ws = 7
    nh = 4
    H = W = max(HW // ws * ws, ws)
    C = max(C0 // nh * nh, nh)
    k = 3
    return {'x': _w((lambda *s: _rng.normal(s) * 0.05)(1, H, W, C)), 'dw_pe': _w((lambda *s: _rng.normal(s) * 0.05)(k, k, C) * 0.1), 'w_qkv': _w((lambda *s: _rng.normal(s) * 0.05)(C, 3 * C) * C ** (-0.5)), 'w_o': _w((lambda *s: _rng.normal(s) * 0.05)(C, C) * C ** (-0.5))}

def reference(x, dw_pe, w_qkv, w_o):
    B, H, W, C = x.shape
    ws = 7
    nh = 4
    dh = C // nh
    kk = dw_pe.shape[0]
    pad = kk // 2
    xp = jnp.pad(x, ((0, 0), (pad, pad), (pad, pad), (0, 0)))
    pe = jnp.zeros_like(x)
    for i in range(kk):
        for j in range(kk):
            pe = pe + xp[:, i:i + H, j:j + W, :] * dw_pe[i, j][None, None, None, :]
    x0 = x + pe
    h = _layernorm(x0, axis=-1)
    hw = h.reshape(B, H // ws, ws, W // ws, ws, C)
    hw = (lambda x, *d: x.transpose(*d))(hw, 0, 1, 3, 2, 4, 5)
    hw = hw.reshape(-1, ws * ws, C)
    qkv = (hw @ w_qkv).reshape(-1, ws * ws, 3, nh, dh)
    q = qkv[:, :, 0].copy()
    k = qkv[:, :, 1].copy()
    v = qkv[:, :, 2].copy()
    scale = dh ** (-0.5)
    attn = jnp.einsum('wnhd,wmhd->whnm', q, k) * scale
    attn = _softmax(attn, axis=-1)
    out = jnp.einsum('whnm,wmhd->wnhd', attn, v)
    out = out.reshape(-1, ws * ws, C) @ w_o
    out = out.reshape(B, H // ws, W // ws, ws, ws, C)
    out = (lambda x, *d: x.transpose(*d))(out, 0, 1, 3, 2, 4, 5)
    out = out.reshape(B, H, W, C)
    return x0 + out
```

```python
import functools
import jax
import jax.numpy as jnp
import jax.experimental.pallas as pl
import jax.experimental.pallas.tpu as pltpu

H = 511
W = 511
WP = 512
C = 192
WS = 7
NW = 73
DH = 48
NEG = -1e30
UNR = 11
SAFE = 30.0
LOG2E = 1.4426950408889634
F32 = jnp.float32
BF16 = jnp.bfloat16


def _iota(shape, dim):
    return jax.lax.broadcasted_iota(jnp.int32, shape, dim)


def _qkv_src(n):
    t = n // 128
    l = n % 128
    t0 = jnp.where(l < 32, 96 + l, l - 32)
    t1 = 192 + t0
    t2 = 384 + jnp.where(l < 96, l, l)
    t3 = jnp.where(l < 64, 384 + 128 + l, 128 + (l - 64))
    t4 = jnp.where(l < 64, -1, 192 + 128 + (l - 64))
    return jnp.where(t == 0, t0, jnp.where(t == 1, t1, jnp.where(t == 2, t2, jnp.where(t == 3, t3, t4))))


def _o_src(n):
    l = n % 128
    a = jnp.where(l < 96, l, -1)
    b = jnp.where(l < 64, 128 + l, jnp.where(l < 96, -1, l))
    return jnp.where(n < 128, a, b)


XR = 9
RING = 16


def _blk_start(s):
    return jnp.clip(s * WS, 0, H - XR)


def _kernel(x_ref, dw_ref, wqkv_ref, wo_ref, out_ref,
            wb_s, wq_s, wo_s, x0a_s, x0_s, h_s, qkv0_s, qkv1_s, o0_s, o1_s, msk_s, p_s, gidx_s):
    s = pl.program_id(0)

    @pl.when(s == 0)
    def _init():
        dw = dw_ref[...].astype(F32)
        for t in range(9):
            col = dw[:, t:t + 1]
            if t == 4:
                col = col + 1.0
            wb_s[t] = jnp.broadcast_to(col, (C, 128))
        n = _iota((576, 640), 1)
        r = _iota((576, 640), 0)
        src = _qkv_src(n)
        pm = jnp.where(r == src, 1.0, 0.0).astype(BF16)
        wq = jnp.dot(wqkv_ref[...], pm, preferred_element_type=F32)
        nn = _iota((C, 640), 1)
        tt = nn // 128
        ll = nn % 128
        isq = (tt == 0) | ((tt == 3) & (ll >= 64))
        wq = jnp.where(isq, wq * (LOG2E * DH ** -0.5), wq)
        wq_s[...] = wq.astype(BF16)
        n2 = _iota((C, 256), 1)
        r2 = _iota((C, 256), 0)
        pm2 = jnp.where(r2 == _o_src(n2), 1.0, 0.0).astype(BF16)
        wot = wo_ref[...].astype(F32).T.astype(BF16)
        wo_s[...] = jnp.dot(wot, pm2, preferred_element_type=F32).astype(BF16)

        l8 = _iota((8, 128), 1)
        s8 = _iota((8, 128), 0)

        def rr(a, b):
            return (l8 >= a) & (l8 < b)

        mk = [
            rr(32, 80), rr(80, 128),
            rr(64, 80) | (l8 < 32), rr(80, 128),
            rr(0, 48) | rr(96, 112), rr(48, 96) | rr(112, 128),
            rr(0, 16) | rr(64, 80) | (l8 >= 96), rr(16, 64) | rr(80, 96),
        ]
        for t in range(8):
            msk_s[t] = jnp.where(mk[t] & ((s8 < 7) | (t < 4)), jnp.uint32(0xFFFFFFFF), jnp.uint32(0))
        wb_s[9] = jnp.zeros((C, 128), F32)
        for ref in (qkv0_s, qkv1_s, o0_s, o1_s):
            ref[...] = jnp.zeros(ref.shape, F32)
        x0_s[...] = jnp.zeros(x0_s.shape, BF16)
        gidx_s[0] = jnp.where(l8 < 48, 96, jnp.where(l8 < 96, 112, l8))
        gidx_s[1] = jnp.where(l8 < 16, 64, jnp.where(l8 < 64, 80, jnp.where(l8 < 96, l8, 64)))


    blk0 = _blk_start(s)

    lane_l = _iota((16, 128), 1) < (W - 3 * 128)

    def conv_groups(R):
        ti = [jnp.where((R + d - 1 >= 0) & (R + d - 1 < H), 3 * d, 9) for d in (0, 2)]
        widx = [ti[0] + jnp.where(ti[0] == 9, 0, t) for t in range(3)] + [3, 4, 5] + \
               [ti[1] + jnp.where(ti[1] == 9, 0, t) for t in range(3)]
        loc = [jnp.clip(R + d - 1 - blk0, 0, XR - 1) for d in range(3)]

        def group(g):
            cs = slice(16 * g, 16 * g + 16)
            rows = []
            for d in range(3):
                v = x_ref[loc[d], cs, :].astype(F32)
                v = jnp.concatenate([v[:, :384], jnp.where(lane_l, v[:, 384:], 0.0)], axis=1)
                rows.append(v)
            w = [jnp.concatenate([wb_s[widx[t], cs, :]] * 4, axis=1) for t in range(9)]
            a = rows[0] * w[0] + rows[1] * w[3] + rows[2] * w[6]
            b = rows[0] * w[1] + rows[1] * w[4] + rows[2] * w[7]
            c = rows[0] * w[2] + rows[1] * w[5] + rows[2] * w[8]
            x0a_s[cs, :] = b + pltpu.roll(a, 1, 1) + pltpu.roll(c, WP - 1, 1)

        return [functools.partial(group, g) for g in range(C // 16)]

    def ln_parts(R):
        slot = R % RING

        def part(hf):
            cb = slice(256 * hf, 256 * hf + 256)
            x0 = x0a_s[:, cb]
            x0_s[slot, :, cb] = x0.astype(BF16)
            mu = jnp.sum(x0, axis=0, keepdims=True) * (1.0 / C)
            d = x0 - mu
            var = jnp.sum(d * d, axis=0, keepdims=True) * (1.0 / C)
            hh = d * jax.lax.rsqrt(var + 1e-5)
            h_s[0, cb, :] = hh[0:128].T.astype(BF16)
            hb = jnp.concatenate([hh[128:192], jnp.zeros((64, 256), F32)], axis=0)
            h_s[1, cb, :] = hb.T.astype(BF16)

        return [functools.partial(part, hf) for hf in range(2)]

    def qkv_parts(qkv_w, r):
        lane = _iota((256, 128), 1)
        lo = lane < 64

        def part(hf):
            cb = slice(256 * hf, 256 * hf + 256)
            y = (jnp.dot(h_s[0, cb, :], wq_s[0:128, :], preferred_element_type=F32)
                 + jnp.dot(h_s[1, cb, 0:64], wq_s[128:192, :], preferred_element_type=F32))
            q0, k0, v0, t3, t4 = [y[:, 128 * t:128 * (t + 1)] for t in range(5)]
            qkv_w[0, r, cb, :] = q0
            qkv_w[1, r, cb, :] = k0
            qkv_w[2, r, cb, :] = jnp.where(lane < 96, v0, 1.0)
            qkv_w[3, r, cb, :] = jnp.where(lo, q0, t3)
            qkv_w[4, r, cb, :] = jnp.where(lo, k0, t4)
            qkv_w[5, r, cb, :] = jnp.where(lo, t3, jnp.where(lane < 96, 1.0, v0))

        return [functools.partial(part, hf) for hf in range(2)]

    def bd(x, m):
        xb = jax.lax.bitcast_convert_type(x, jnp.uint32).reshape(8, 8, 128)
        xa_ = (xb & msk_s[2 * m][None]).reshape(64, 128)
        xc_ = (xb & msk_s[2 * m + 1][None]).reshape(64, 128)
        xx = jax.lax.bitcast_convert_type(jnp.concatenate([xa_, xc_], axis=0), F32)
        return xx.astype(BF16)

    def ldw(qkv_r, t, base):
        return qkv_r[t, :, pl.ds(base, 8), :].reshape(64, 128)

    def scores(qkv_r, p, base):
        return jax.lax.dot_general(ldw(qkv_r, 3 * p, base).astype(BF16), bd(ldw(qkv_r, 3 * p + 1, base), p),
                                   (((1,), (1,)), ((), ())), preferred_element_type=F32)

    gis = [gidx_s[0], gidx_s[1]]

    def pv(qkv_r, o_w, pr, p, base):
        o = jnp.dot(pr, bd(ldw(qkv_r, 3 * p + 2, base), 2 + p), preferred_element_type=F32)
        o = o.reshape(8, 8, 128)
        for i in range(8):
            oi = o[i]
            den = jnp.take_along_axis(oi, gis[p], axis=1)
            o_w[p, i, pl.ds(base, 8), :] = oi * pl.reciprocal(den, approx=True)

    def out_parts(o_r, R, r):
        slot = R % RING

        def part(hf):
            cb = slice(256 * hf, 256 * hf + 256)
            ob = jnp.concatenate([o_r[0, r, cb, :], o_r[1, r, cb, :]], axis=1).astype(BF16)
            y = jax.lax.dot_general(wo_s[...], ob, (((1,), (1,)), ((), ())),
                                    preferred_element_type=F32)
            out_ref[r, :, cb] = (x0_s[slot, :, cb].astype(F32) + y).astype(BF16)

        return [functools.partial(part, hf) for hf in range(2)]

    def interleave(*lists):
        n = max(len(l) for l in lists)
        items = []
        for li, l in enumerate(lists):
            for i, f in enumerate(l):
                items.append(((i + 0.5) / len(l), li, f))
        for _, _, f in sorted(items, key=lambda t: (t[0], t[1])):
            f()

    @pl.when(s == 0)
    def _prologue():
        for f in conv_groups(0) + ln_parts(0):
            f()

    def step(qkv_w, qkv_r, o_w, o_r):
        def body(r, amax_in):
            R = s * WS + r
            bases = [jnp.minimum(r * UNR + u, NW - 1) * WS for u in range(UNR)]
            am = [amax_in]

            def c1(p, u):
                sc = scores(qkv_r, p, bases[u])
                am[0] = jnp.maximum(am[0], jnp.max(jnp.abs(sc).reshape(8, 8, 128), axis=0))
                p_s[p, u] = jnp.exp2(sc).astype(BF16)

            def c2(p, u):
                pv(qkv_r, o_w, p_s[p, u], p, bases[u])

            c1s = [functools.partial(c1, p, u) for p in range(2) for u in range(UNR)]
            c2s = [functools.partial(c2, p, u) for p in range(2) for u in range(UNR)]
            cv = conv_groups(R + 1)
            ln = ln_parts(R + 1)
            qk = qkv_parts(qkv_w, r)
            ou = out_parts(o_r, R + RING - 2 * WS, r)
            interleave(qk, c1s, cv)
            interleave(ou, c2s, ln)
            return am[0]

        amax = jax.lax.fori_loop(0, WS, functools.partial(body), jnp.zeros((8, 128), F32))

        @pl.when(jnp.logical_not(jnp.max(amax) <= SAFE))
        def _safe_softmax():
            l8 = _iota((8, 128), 1)
            kvalid = ((l8 % 8) != 7) & ((l8 % 64) < 56)
            ba = jnp.where(kvalid & (l8 < 64), 0.0, NEG)[None]
            bb = jnp.where(kvalid & (l8 >= 64), 0.0, NEG)[None]

            def one(j, carry):
                for p in range(2):
                    sc = scores(qkv_r, p, j * WS).reshape(8, 8, 128)
                    s_a = sc + ba
                    s_b = sc + bb
                    d = jnp.maximum(s_a - jnp.max(s_a, axis=2, keepdims=True),
                                    s_b - jnp.max(s_b, axis=2, keepdims=True))
                    pv(qkv_r, o_w, jnp.exp2(d).reshape(64, 128).astype(BF16), p, j * WS)
                return carry

            jax.lax.fori_loop(0, NW, one, 0)


    @pl.when(s % 2 == 0)
    def _even():
        step(qkv0_s, qkv1_s, o0_s, o1_s)

    @pl.when(s % 2 == 1)
    def _odd():
        step(qkv1_s, qkv0_s, o1_s, o0_s)


@jax.jit
def pallas_standalone__window_attn_davit__vision_kernel(x, dw_pe, w_qkv, w_o):
    xt = jnp.transpose(x.reshape(H, W, C), (0, 2, 1))
    dwt = jnp.transpose(dw_pe.reshape(9, C), (1, 0))
    out = pl.pallas_call(
        _kernel,
        grid=(NW + 2,),
        in_specs=[
            pl.BlockSpec((pl.Element(XR), pl.Element(C), pl.Element(WP, (0, 1))),
                         lambda s: (_blk_start(s), 0, 0)),
            pl.BlockSpec((C, 9), lambda s: (0, 0)),
            pl.BlockSpec((C, 3 * C), lambda s: (0, 0)),
            pl.BlockSpec((C, C), lambda s: (0, 0)),
        ],
        out_specs=pl.BlockSpec((WS, C, WP), lambda s: (jnp.maximum(s - 2, 0), 0, 0)),
        out_shape=jax.ShapeDtypeStruct((H, C, W), BF16),
        scratch_shapes=[
            pltpu.VMEM((10, C, 128), F32),
            pltpu.VMEM((C, 640), BF16),
            pltpu.VMEM((C, 256), BF16),
            pltpu.VMEM((C, WP), F32),
            pltpu.VMEM((RING, C, WP), BF16),
            pltpu.VMEM((2, WP, 128), BF16),
            pltpu.VMEM((6, 8, WP, 128), F32),
            pltpu.VMEM((6, 8, WP, 128), F32),
            pltpu.VMEM((2, 8, WP, 128), F32),
            pltpu.VMEM((2, 8, WP, 128), F32),
            pltpu.VMEM((8, 8, 128), jnp.uint32),
            pltpu.VMEM((2, UNR, 64, 128), BF16),
            pltpu.VMEM((2, 8, 128), jnp.int32),
        ],
        compiler_params=pltpu.CompilerParams(
            dimension_semantics=("arbitrary",),
            vmem_limit_bytes=100 * 2**20,
        ),
    )(xt, dwt, w_qkv, w_o)
    return jnp.transpose(out, (0, 2, 1)).reshape(1, H, W, C)
```

```python
import functools
import jax
import jax.numpy as jnp
import jax.experimental.pallas as pl
import jax.experimental.pallas.tpu as pltpu

H = 511
W = 511
WP = 512
C = 192
WS = 7
NW = 73
DH = 48
NEG = -1e30
UNR = 11
QM = 128
SAFE = 30.0
LOG2E = 1.4426950408889634
F32 = jnp.float32
BF16 = jnp.bfloat16


def _iota(shape, dim):
    return jax.lax.broadcasted_iota(jnp.int32, shape, dim)


def _qkv_src(n):
    t = n // 128
    l = n % 128
    t0 = jnp.where(l < 32, 96 + l, l - 32)
    t1 = 192 + t0
    t2 = 384 + jnp.where(l < 96, l, l)
    t3 = jnp.where(l < 64, 384 + 128 + l, 128 + (l - 64))
    t4 = jnp.where(l < 64, -1, 192 + 128 + (l - 64))
    return jnp.where(t == 0, t0, jnp.where(t == 3, t1, jnp.where(t == 1, t2, jnp.where(t == 2, t3, t4))))


def _o_src(n):
    l = n % 128
    a = jnp.where(l < 96, l, -1)
    b = jnp.where(l < 64, 128 + l, jnp.where(l < 96, -1, l))
    return jnp.where(n < 128, a, b)


XR = 9
RING = 16


def _blk_start(s):
    return jnp.clip(s * WS, 0, H - XR)


def _b2u(x):
    return pltpu.bitcast(x, jnp.uint32)


def _u2b(x):
    return pltpu.bitcast(x, BF16)


def _kernel(x_ref, dw_ref, wqkv_ref, wo_ref, out_ref,
            wb_s, wq_s, wo_s, x0_s, h_s, qkv0_s, qkv1_s, o0_s, o1_s, msk_s, p_s, gidx_s):
    s = pl.program_id(0)

    @pl.when(s == 0)
    def _init():
        dw = dw_ref[...].astype(F32)
        for t in range(9):
            col = dw[:, t:t + 1]
            if t == 4:
                col = col + 1.0
            wb_s[t] = jnp.broadcast_to(col, (C, 128))
        n = _iota((576, 640), 1)
        r = _iota((576, 640), 0)
        src = _qkv_src(n)
        pm = jnp.where(r == src, 1.0, 0.0).astype(BF16)
        wq = jnp.dot(wqkv_ref[...], pm, preferred_element_type=F32)
        nn = _iota((C, 640), 1)
        tt = nn // 128
        ll = nn % 128
        isq = (tt == 0) | ((tt == 2) & (ll >= 64))
        wq = jnp.where(isq, wq * (LOG2E * DH ** -0.5), wq)
        wq_s[...] = _b2u(wq.astype(BF16))
        n2 = _iota((C, 256), 1)
        r2 = _iota((C, 256), 0)
        pm2 = jnp.where(r2 == _o_src(n2), 1.0, 0.0).astype(BF16)
        wot = wo_ref[...].astype(F32).T.astype(BF16)
        wo_s[...] = _b2u(jnp.dot(wot, pm2, preferred_element_type=F32).astype(BF16))

        l8 = _iota((8, 128), 1)
        s8 = _iota((8, 128), 0)

        def rr(a, b):
            return (l8 >= a) & (l8 < b)

        mk = [
            rr(32, 80), rr(80, 128),
            rr(64, 80) | (l8 < 32), rr(80, 128),
            rr(0, 48) | rr(96, 112), rr(48, 96) | rr(112, 128),
            rr(0, 16) | rr(64, 80) | (l8 >= 96), rr(16, 64) | rr(80, 96),
        ]
        for t in range(8):
            msk_s[t] = jnp.where(mk[t] & ((s8 < 7) | (t < 4)), jnp.uint32(0xFFFFFFFF), jnp.uint32(0))
        wb_s[9] = jnp.zeros((C, 128), F32)
        for ref in (qkv0_s, qkv1_s):
            for t in range(6):
                ref[t, 7] = jnp.zeros((WP, 128), F32)
        gidx_s[0] = jnp.where(l8 < 48, 96, jnp.where(l8 < 96, 112, l8))
        gidx_s[1] = jnp.where(l8 < 16, 64, jnp.where(l8 < 64, 80, jnp.where(l8 < 96, l8, 64)))


    blk0 = _blk_start(s)

    lane_l = _iota((8, 128), 1) < (W - 3 * 128)

    def conv_groups(R):
        ti = [jnp.where((R + d - 1 >= 0) & (R + d - 1 < H), 3 * d, 9) for d in (0, 2)]
        widx = [ti[0] + jnp.where(ti[0] == 9, 0, t) for t in range(3)] + [3, 4, 5] + \
               [ti[1] + jnp.where(ti[1] == 9, 0, t) for t in range(3)]
        loc = [jnp.clip(R + d - 1 - blk0, 0, XR - 1) for d in range(3)]

        slot = R % RING

        def half(g):
            cs = slice(8 * g, 8 * g + 8)
            rows = []
            for d in range(3):
                v = x_ref[loc[d], cs, :].astype(F32)
                v = jnp.concatenate([v[:, :384], jnp.where(lane_l, v[:, 384:], 0.0)], axis=1)
                rows.append(v)
            w = [jnp.concatenate([wb_s[widx[t], cs, :]] * 4, axis=1) for t in range(9)]
            a = rows[0] * w[0] + rows[1] * w[3] + rows[2] * w[6]
            b = rows[0] * w[1] + rows[1] * w[4] + rows[2] * w[7]
            c = rows[0] * w[2] + rows[1] * w[5] + rows[2] * w[8]
            return b + pltpu.roll(a, 1, 1) + pltpu.roll(c, WP - 1, 1)

        def group(g):
            x0 = jnp.concatenate([half(2 * g), half(2 * g + 1)], axis=0)
            x0_s[slot, 16 * g:16 * g + 16, :] = x0.astype(BF16)

        return [functools.partial(group, g) for g in range(C // 16)]

    def ln_parts(R):
        slot = R % RING

        def part(hf):
            cb = slice(256 * hf, 256 * hf + 256)
            x0 = x0_s[slot, :, cb].astype(F32)
            mu = jnp.sum(x0, axis=0, keepdims=True) * (1.0 / C)
            d = x0 - mu
            var = jnp.sum(d * d, axis=0, keepdims=True) * (1.0 / C)
            hh = d * jax.lax.rsqrt(var + 1e-5)
            h_s[0, cb, :] = hh[0:128].T.astype(BF16)
            hb = jnp.concatenate([hh[128:192], jnp.zeros((64, 256), F32)], axis=0)
            h_s[1, cb, :] = hb.T.astype(BF16)

        return [functools.partial(part, hf) for hf in range(2)]

    def qkv_parts(qkv_w, r):
        lane = _iota((QM, 128), 1)
        lo = lane < 64

        def mm(cb, t0, t1):
            c2 = slice(cb.start // 2, cb.stop // 2)
            ns = slice(128 * t0, 128 * t1)
            return (jnp.dot(h_s[0, cb, :], _u2b(wq_s[0:64, ns]), preferred_element_type=F32)
                    + jnp.dot(h_s[1, cb, 0:64], _u2b(wq_s[64:96, ns]), preferred_element_type=F32))

        def part_a(hf):
            cb = slice(QM * hf, QM * hf + QM)
            y = mm(cb, 0, 3)
            q0, v0, t3 = [y[:, 128 * t:128 * (t + 1)] for t in range(3)]
            qkv_w[0, r, cb, :] = q0
            qkv_w[2, r, cb, :] = jnp.where(lane < 96, v0, 1.0)
            qkv_w[3, r, cb, :] = jnp.where(lo, q0, t3)
            qkv_w[5, r, cb, :] = jnp.where(lo, t3, jnp.where(lane < 96, 1.0, v0))

        def part_b(hf):
            cb = slice(QM * hf, QM * hf + QM)
            y = mm(cb, 3, 5)
            k0, t4 = [y[:, 128 * t:128 * (t + 1)] for t in range(2)]
            qkv_w[1, r, cb, :] = k0
            qkv_w[4, r, cb, :] = jnp.where(lo, k0, t4)

        return [functools.partial(f, hf) for hf in range(WP // QM) for f in (part_a, part_b)]

    def bd(x, m):
        xb = jax.lax.bitcast_convert_type(x, jnp.uint32).reshape(8, 8, 128)
        xa_ = (xb & msk_s[2 * m][None]).reshape(64, 128)
        xc_ = (xb & msk_s[2 * m + 1][None]).reshape(64, 128)
        xx = jax.lax.bitcast_convert_type(jnp.concatenate([xa_, xc_], axis=0), F32)
        return xx.astype(BF16)

    def ldw(qkv_r, t, base):
        return qkv_r[t, :, pl.ds(base, 8), :].reshape(64, 128)

    def scores(qkv_r, p, base):
        return jax.lax.dot_general(ldw(qkv_r, 3 * p, base).astype(BF16), bd(ldw(qkv_r, 3 * p + 1, base), p),
                                   (((1,), (1,)), ((), ())), preferred_element_type=F32)

    gis = [gidx_s[0], gidx_s[1]]

    def pv(qkv_r, o_w, pr, p, base):
        o = jnp.dot(pr, bd(ldw(qkv_r, 3 * p + 2, base), 2 + p), preferred_element_type=F32)
        o = o.reshape(8, 8, 128)
        gi = gis[p]
        for i in range(8):
            oi = o[i]
            den = jnp.take_along_axis(oi, gi, axis=1)
            o_w[p, i, pl.ds(base, 8), :] = oi * pl.reciprocal(den, approx=True)

    def out_parts(o_r, R, r):
        slot = R % RING

        def part(hf):
            cb = slice(256 * hf, 256 * hf + 256)
            ob = jnp.concatenate([o_r[0, r, cb, :], o_r[1, r, cb, :]], axis=1).astype(BF16)
            y = jax.lax.dot_general(_u2b(wo_s[...]), ob, (((1,), (1,)), ((), ())),
                                    preferred_element_type=F32)
            out_ref[r, :, cb] = (x0_s[slot, :, cb].astype(F32) + y).astype(BF16)

        return [functools.partial(part, hf) for hf in range(2)]

    @pl.when(s == 0)
    def _prologue():
        for f in conv_groups(0) + ln_parts(0):
            f()

    def step(qkv_w, qkv_r, o_w, o_r, do_ab, do_c, do_d):
        def body(r, amax_in):
            R = s * WS + r
            am = [amax_in]
            units = [(p, jnp.minimum(r * UNR + u, NW - 1) * WS) for p in range(2) for u in range(UNR)]

            def c1(u):
                p, base = units[u]
                sc = scores(qkv_r, p, base)
                am[0] = jnp.maximum(am[0], jnp.max(jnp.abs(sc).reshape(8, 8, 128), axis=0))
                p_s[u] = jnp.exp2(sc).astype(BF16)

            def c2(u):
                p, base = units[u]
                pv(qkv_r, o_w, p_s[u], p, base)

            work = []
            if do_ab:
                work += qkv_parts(qkv_w, r) + conv_groups(R + 1)
            if do_c:
                work += [functools.partial(c1, u) for u in range(2 * UNR)]
            if do_ab:
                work += ln_parts(R + 1)
            if do_c:
                work += [functools.partial(c2, u) for u in range(2 * UNR)]
            if do_d:
                work += out_parts(o_r, R + RING - 2 * WS, r)
            for f in work:
                f()
            return am[0]

        amax = jax.lax.fori_loop(0, WS, body, jnp.zeros((8, 128), F32))
        if not do_c:
            return

        @pl.when(jnp.logical_not(jnp.max(amax) <= SAFE))
        def _safe_softmax():
            l8 = _iota((8, 128), 1)
            kvalid = ((l8 % 8) != 7) & ((l8 % 64) < 56)
            ba = jnp.where(kvalid & (l8 < 64), 0.0, NEG)[None]
            bb = jnp.where(kvalid & (l8 >= 64), 0.0, NEG)[None]

            def one(j, carry):
                for p in range(2):
                    sc = scores(qkv_r, p, j * WS).reshape(8, 8, 128)
                    s_a = sc + ba
                    s_b = sc + bb
                    d = jnp.maximum(s_a - jnp.max(s_a, axis=2, keepdims=True),
                                    s_b - jnp.max(s_b, axis=2, keepdims=True))
                    pv(qkv_r, o_w, jnp.exp2(d).reshape(64, 128).astype(BF16), p, j * WS)
                return carry

            jax.lax.fori_loop(0, NW, one, 0)

    even = (qkv0_s, qkv1_s, o0_s, o1_s)
    odd = (qkv1_s, qkv0_s, o1_s, o0_s)
    main = (s >= 2) & (s < NW)
    pl.when(s == 0)(lambda: step(*even, True, False, False))
    pl.when(s == 1)(lambda: step(*odd, True, True, False))
    pl.when(main & (s % 2 == 0))(lambda: step(*even, True, True, True))
    pl.when(main & (s % 2 == 1))(lambda: step(*odd, True, True, True))
    pl.when(s == NW)(lambda: step(*(odd if NW % 2 else even), False, True, True))
    pl.when(s == NW + 1)(lambda: step(*(even if NW % 2 else odd), False, False, True))


@jax.jit
def pallas_standalone__window_attn_davit__vision_kernel(x, dw_pe, w_qkv, w_o):
    xt = jnp.transpose(x.reshape(H, W, C), (0, 2, 1))
    dwt = jnp.transpose(dw_pe.reshape(9, C), (1, 0))
    out = pl.pallas_call(
        _kernel,
        grid=(NW + 2,),
        in_specs=[
            pl.BlockSpec((pl.Element(XR), pl.Element(C), pl.Element(WP, (0, 1))),
                         lambda s: (_blk_start(s), 0, 0)),
            pl.BlockSpec((C, 9), lambda s: (0, 0)),
            pl.BlockSpec((C, 3 * C), lambda s: (0, 0)),
            pl.BlockSpec((C, C), lambda s: (0, 0)),
        ],
        out_specs=pl.BlockSpec((WS, C, WP), lambda s: (jnp.maximum(s - 2, 0), 0, 0)),
        out_shape=jax.ShapeDtypeStruct((H, C, W), BF16),
        scratch_shapes=[
            pltpu.VMEM((10, C, 128), F32),
            pltpu.VMEM((C // 2, 640), jnp.uint32),
            pltpu.VMEM((C // 2, 256), jnp.uint32),
            pltpu.VMEM((RING, C, WP), BF16),
            pltpu.VMEM((2, WP, 128), BF16),
            pltpu.VMEM((6, 8, WP, 128), F32),
            pltpu.VMEM((6, 8, WP, 128), F32),
            pltpu.VMEM((2, 8, WP, 128), F32),
            pltpu.VMEM((2, 8, WP, 128), F32),
            pltpu.VMEM((8, 8, 128), jnp.uint32),
            pltpu.VMEM((2 * UNR, 64, 128), BF16),
            pltpu.VMEM((2, 8, 128), jnp.int32),
        ],
        compiler_params=pltpu.CompilerParams(
            dimension_semantics=("arbitrary",),
            vmem_limit_bytes=100 * 2**20,
        ),
    )(xt, dwt, w_qkv, w_o)
    return jnp.transpose(out, (0, 2, 1)).reshape(1, H, W, C)
```

```python
import functools
import jax
import jax.numpy as jnp
import jax.experimental.pallas as pl
import jax.experimental.pallas.tpu as pltpu

H = 511
W = 511
WP = 512
C = 192
WS = 7
NW = 73
DH = 48
NEG = -1e30
UNR = 11
QM = 256
SAFE = 30.0
LOG2E = 1.4426950408889634
F32 = jnp.float32
BF16 = jnp.bfloat16


def _iota(shape, dim):
    return jax.lax.broadcasted_iota(jnp.int32, shape, dim)


def _qkv_src(n):
    t = n // 128
    l = n % 128
    t0 = jnp.where(l < 32, 96 + l, l - 32)
    t1 = 192 + t0
    t2 = 384 + jnp.where(l < 96, l, l)
    t3 = jnp.where(l < 64, 384 + 128 + l, 128 + (l - 64))
    t4 = jnp.where(l < 64, -1, 192 + 128 + (l - 64))
    return jnp.where(t == 0, t0, jnp.where(t == 3, t1, jnp.where(t == 1, t2, jnp.where(t == 2, t3, t4))))


def _o_src(n):
    l = n % 128
    a = jnp.where(l < 96, l, -1)
    b = jnp.where(l < 64, 128 + l, jnp.where(l < 96, -1, l))
    return jnp.where(n < 128, a, b)


XR = 9
RING = 16


def _blk_start(s):
    return jnp.clip(s * WS, 0, H - XR)


def _b2u(x):
    return pltpu.bitcast(x, jnp.uint32)


def _u2b(x):
    return pltpu.bitcast(x, BF16)


def _kernel(x_ref, dw_ref, wqkv_ref, wo_ref, out_ref,
            wb_s, wq_s, wo_s, x0_s, h_s, qkv0_s, qkv1_s, o0_s, o1_s, msk_s, p_s, gidx_s):
    s = pl.program_id(0)

    @pl.when(s == 0)
    def _init():
        dw = dw_ref[...].astype(F32)
        for t in range(9):
            col = dw[:, t:t + 1]
            if t == 4:
                col = col + 1.0
            wb_s[t] = jnp.broadcast_to(col, (C, 128))
        n = _iota((576, 640), 1)
        r = _iota((576, 640), 0)
        src = _qkv_src(n)
        pm = jnp.where(r == src, 1.0, 0.0).astype(BF16)
        wq = jnp.dot(wqkv_ref[...], pm, preferred_element_type=F32)
        nn = _iota((C, 640), 1)
        tt = nn // 128
        ll = nn % 128
        isq = (tt == 0) | ((tt == 2) & (ll >= 64))
        wq = jnp.where(isq, wq * (LOG2E * DH ** -0.5), wq)
        wq_s[...] = _b2u(wq.astype(BF16))
        n2 = _iota((C, 256), 1)
        r2 = _iota((C, 256), 0)
        pm2 = jnp.where(r2 == _o_src(n2), 1.0, 0.0).astype(BF16)
        wot = wo_ref[...].astype(F32).T.astype(BF16)
        wo_s[...] = _b2u(jnp.dot(wot, pm2, preferred_element_type=F32).astype(BF16))

        l8 = _iota((8, 128), 1)
        s8 = _iota((8, 128), 0)

        def rr(a, b):
            return (l8 >= a) & (l8 < b)

        mk = [
            rr(32, 80), rr(80, 128),
            rr(64, 80) | (l8 < 32), rr(80, 128),
            rr(0, 48) | rr(96, 112), rr(48, 96) | rr(112, 128),
            rr(0, 16) | rr(64, 80) | (l8 >= 96), rr(16, 64) | rr(80, 96),
        ]
        for t in range(8):
            msk_s[t] = jnp.where(mk[t] & ((s8 < 7) | (t < 4)), jnp.uint32(0xFFFFFFFF), jnp.uint32(0))
        wb_s[9] = jnp.zeros((C, 128), F32)
        for ref in (qkv0_s, qkv1_s):
            for t in range(6):
                ref[t, 7] = jnp.zeros((WP, 128), F32)
        gidx_s[0] = jnp.where(l8 < 48, 96, jnp.where(l8 < 96, 112, l8))
        gidx_s[1] = jnp.where(l8 < 16, 64, jnp.where(l8 < 64, 80, jnp.where(l8 < 96, l8, 64)))


    blk0 = _blk_start(s)

    def conv_groups(R):
        ti = [jnp.where((R + d - 1 >= 0) & (R + d - 1 < H), 3 * d, 9) for d in (0, 2)]
        widx = [ti[0] + jnp.where(ti[0] == 9, 0, t) for t in range(3)] + [3, 4, 5] + \
               [ti[1] + jnp.where(ti[1] == 9, 0, t) for t in range(3)]
        loc = [jnp.clip(R + d - 1 - blk0, 0, XR - 1) for d in range(3)]

        slot = R % RING

        def half(g):
            cs = slice(8 * g, 8 * g + 8)
            rows = []
            for d in range(3):
                v = x_ref[loc[d], cs, :].astype(F32)
                v = jnp.concatenate([v[:, :384], jnp.pad(v[:, 384:], ((0, 0), (0, 1)))], axis=1)
                rows.append(v)
            w = [jnp.concatenate([wb_s[widx[t], cs, :]] * 4, axis=1) for t in range(9)]
            a = rows[0] * w[0] + rows[1] * w[3] + rows[2] * w[6]
            b = rows[0] * w[1] + rows[1] * w[4] + rows[2] * w[7]
            c = rows[0] * w[2] + rows[1] * w[5] + rows[2] * w[8]
            return b + pltpu.roll(a, 1, 1) + pltpu.roll(c, WP - 1, 1)

        def group(g):
            x0 = jnp.concatenate([half(2 * g), half(2 * g + 1)], axis=0)
            x0_s[slot, 16 * g:16 * g + 16, :] = x0.astype(BF16)

        return [functools.partial(group, g) for g in range(C // 16)]

    def ln_parts(R):
        slot = R % RING

        def part(hf):
            cb = slice(256 * hf, 256 * hf + 256)
            x0 = x0_s[slot, :, cb].astype(F32)
            mu = jnp.sum(x0, axis=0, keepdims=True) * (1.0 / C)
            d = x0 - mu
            var = jnp.sum(d * d, axis=0, keepdims=True) * (1.0 / C)
            hh = d * jax.lax.rsqrt(var + 1e-5)
            h_s[0, cb, :] = hh[0:128].T.astype(BF16)
            hb = jnp.concatenate([hh[128:192], jnp.zeros((64, 256), F32)], axis=0)
            h_s[1, cb, :] = hb.T.astype(BF16)

        return [functools.partial(part, hf) for hf in range(2)]

    def qkv_parts(qkv_w, r):
        lane = _iota((QM, 128), 1)
        lo = lane < 64

        def mm(cb, t0, t1):
            c2 = slice(cb.start // 2, cb.stop // 2)
            ns = slice(128 * t0, 128 * t1)
            return (jnp.dot(h_s[0, cb, :], _u2b(wq_s[0:64, ns]), preferred_element_type=F32)
                    + jnp.dot(h_s[1, cb, 0:64], _u2b(wq_s[64:96, ns]), preferred_element_type=F32))

        def part_a(hf):
            cb = slice(QM * hf, QM * hf + QM)
            y = mm(cb, 0, 3)
            q0, v0, t3 = [y[:, 128 * t:128 * (t + 1)] for t in range(3)]
            qkv_w[0, r, cb, :] = q0
            qkv_w[2, r, cb, :] = jnp.where(lane < 96, v0, 1.0)
            qkv_w[3, r, cb, :] = jnp.where(lo, q0, t3)
            qkv_w[5, r, cb, :] = jnp.where(lo, t3, jnp.where(lane < 96, 1.0, v0))

        def part_b(hf):
            cb = slice(QM * hf, QM * hf + QM)
            y = mm(cb, 3, 5)
            k0, t4 = [y[:, 128 * t:128 * (t + 1)] for t in range(2)]
            qkv_w[1, r, cb, :] = k0
            qkv_w[4, r, cb, :] = jnp.where(lo, k0, t4)

        return [functools.partial(f, hf) for hf in range(WP // QM) for f in (part_a, part_b)]

    def bd(x, m):
        xb = jax.lax.bitcast_convert_type(x, jnp.uint32).reshape(8, 8, 128)
        xa_ = (xb & msk_s[2 * m][None]).reshape(64, 128)
        xc_ = (xb & msk_s[2 * m + 1][None]).reshape(64, 128)
        xx = jax.lax.bitcast_convert_type(jnp.concatenate([xa_, xc_], axis=0), F32)
        return xx.astype(BF16)

    def ldw(qkv_r, t, base):
        return qkv_r[t, :, pl.ds(base, 8), :].reshape(64, 128)

    def scores(qkv_r, p, base):
        return jax.lax.dot_general(ldw(qkv_r, 3 * p, base).astype(BF16), bd(ldw(qkv_r, 3 * p + 1, base), p),
                                   (((1,), (1,)), ((), ())), preferred_element_type=F32)

    gis = [gidx_s[0], gidx_s[1]]

    def pv(qkv_r, o_w, pr, p, base):
        o = jnp.dot(pr, bd(ldw(qkv_r, 3 * p + 2, base), 2 + p), preferred_element_type=F32)
        o = o.reshape(8, 8, 128)
        gi = gis[p]
        for i in range(8):
            oi = o[i]
            den = jnp.take_along_axis(oi, gi, axis=1)
            o_w[p, i, pl.ds(base, 8), :] = oi * pl.reciprocal(den, approx=True)

    def out_parts(o_r, R, r):
        slot = R % RING

        def part(hf):
            cb = slice(256 * hf, 256 * hf + 256)
            ob = jnp.concatenate([o_r[0, r, cb, :], o_r[1, r, cb, :]], axis=1).astype(BF16)
            y = jax.lax.dot_general(_u2b(wo_s[...]), ob, (((1,), (1,)), ((), ())),
                                    preferred_element_type=F32)
            out_ref[r, :, cb] = (x0_s[slot, :, cb].astype(F32) + y).astype(BF16)

        return [functools.partial(part, hf) for hf in range(2)]

    @pl.when(s == 0)
    def _prologue():
        for f in conv_groups(0) + ln_parts(0):
            f()

    def step(qkv_w, qkv_r, o_w, o_r, do_ab, do_c, do_d):
        def body(r, amax_in, nw=UNR, w0=None):
            R = s * WS + r
            am = [amax_in]
            if w0 is None:
                units = [(p, jnp.minimum(r * UNR + u, NW - 1) * WS) for p in range(2) for u in range(UNR)]
            else:
                units = [(p, (w0 + u) * WS) for p in range(2) for u in range(nw)]

            def c1(u):
                p, base = units[u]
                sc = scores(qkv_r, p, base)
                am[0] = jnp.maximum(am[0], jnp.max(jnp.abs(sc).reshape(8, 8, 128), axis=0))
                p_s[u] = jnp.exp2(sc).astype(BF16)

            def c2(u):
                p, base = units[u]
                pv(qkv_r, o_w, p_s[u], p, base)

            c2s = [functools.partial(c2, u) for u in range(2 * nw)] if do_c else []
            cut = int(0.4 * len(c2s))
            work = []
            if do_ab:
                work += qkv_parts(qkv_w, r) + conv_groups(R + 1)
            if do_c:
                work += [functools.partial(c1, u) for u in range(2 * nw)]
            work += c2s[:cut]
            if do_ab:
                work += ln_parts(R + 1)
            work += c2s[cut:]
            if do_d:
                work += out_parts(o_r, R + RING - 2 * WS, r)
            for f in work:
                f()
            return jnp.broadcast_to(jnp.max(am[0], axis=(0, 1), keepdims=True), (8, 128)) if do_c else am[0]

        def body_split(r, amax_in):
            w0 = 10 * r + jnp.minimum((r + 1) // 2, 3)
            return jax.lax.cond((r % 2 == 0) & (r < 6),
                                lambda: body(r, amax_in, 11, w0),
                                lambda: body(r, amax_in, 10, w0))

        full = do_ab and do_c and do_d
        amax = jax.lax.fori_loop(0, WS, body_split if full else body, jnp.zeros((8, 128), F32))
        if not do_c:
            return

        @pl.when(jnp.logical_not(amax[0, 0] <= SAFE))
        def _safe_softmax():
            l8 = _iota((8, 128), 1)
            kvalid = ((l8 % 8) != 7) & ((l8 % 64) < 56)
            ba = jnp.where(kvalid & (l8 < 64), 0.0, NEG)[None]
            bb = jnp.where(kvalid & (l8 >= 64), 0.0, NEG)[None]

            def one(j, carry):
                for p in range(2):
                    sc = scores(qkv_r, p, j * WS).reshape(8, 8, 128)
                    s_a = sc + ba
                    s_b = sc + bb
                    d = jnp.maximum(s_a - jnp.max(s_a, axis=2, keepdims=True),
                                    s_b - jnp.max(s_b, axis=2, keepdims=True))
                    pv(qkv_r, o_w, jnp.exp2(d).reshape(64, 128).astype(BF16), p, j * WS)
                return carry

            jax.lax.fori_loop(0, NW, one, 0)

    even = (qkv0_s, qkv1_s, o0_s, o1_s)
    odd = (qkv1_s, qkv0_s, o1_s, o0_s)
    main = (s >= 2) & (s < NW)
    pl.when(s == 0)(lambda: step(*even, True, False, False))
    pl.when(s == 1)(lambda: step(*odd, True, True, False))
    pl.when(main & (s % 2 == 0))(lambda: step(*even, True, True, True))
    pl.when(main & (s % 2 == 1))(lambda: step(*odd, True, True, True))
    pl.when(s == NW)(lambda: step(*(odd if NW % 2 else even), False, True, True))
    pl.when(s == NW + 1)(lambda: step(*(even if NW % 2 else odd), False, False, True))


@jax.jit
def pallas_standalone__window_attn_davit__vision_kernel(x, dw_pe, w_qkv, w_o):
    xt = jnp.transpose(x.reshape(H, W, C), (0, 2, 1))
    dwt = jnp.transpose(dw_pe.reshape(9, C), (1, 0))
    out = pl.pallas_call(
        _kernel,
        grid=(NW + 2,),
        in_specs=[
            pl.BlockSpec((pl.Element(XR), pl.Element(C), pl.Element(W)),
                         lambda s: (_blk_start(s), 0, 0)),
            pl.BlockSpec((C, 9), lambda s: (0, 0)),
            pl.BlockSpec((C, 3 * C), lambda s: (0, 0)),
            pl.BlockSpec((C, C), lambda s: (0, 0)),
        ],
        out_specs=pl.BlockSpec((WS, C, WP), lambda s: (jnp.maximum(s - 2, 0), 0, 0)),
        out_shape=jax.ShapeDtypeStruct((H, C, W), BF16),
        scratch_shapes=[
            pltpu.VMEM((10, C, 128), F32),
            pltpu.VMEM((C // 2, 640), jnp.uint32),
            pltpu.VMEM((C // 2, 256), jnp.uint32),
            pltpu.VMEM((RING, C, WP), BF16),
            pltpu.VMEM((2, WP, 128), BF16),
            pltpu.VMEM((6, 8, WP, 128), F32),
            pltpu.VMEM((6, 8, WP, 128), F32),
            pltpu.VMEM((2, 8, WP, 128), F32),
            pltpu.VMEM((2, 8, WP, 128), F32),
            pltpu.VMEM((8, 8, 128), jnp.uint32),
            pltpu.VMEM((2 * UNR, 64, 128), BF16),
            pltpu.VMEM((2, 8, 128), jnp.int32),
        ],
        compiler_params=pltpu.CompilerParams(
            dimension_semantics=("arbitrary",),
            vmem_limit_bytes=100 * 2**20,
        ),
    )(xt, dwt, w_qkv, w_o)
    return jnp.transpose(out, (0, 2, 1)).reshape(1, H, W, C)
```
